```python
import os as _os
_os.environ.setdefault("JAX_PLATFORMS", "cpu")
import jax
import jax.numpy as jnp

def _softmax(x, axis=-1):
    return jax.nn.softmax(x, axis=axis)
def _gelu(x):
    return jax.nn.gelu(x, approximate=True)
def _silu(x):
    return jax.nn.silu(x)
def _sigmoid(x):
    return jax.nn.sigmoid(x)
def _layernorm(x, axis=-1, eps=1e-5):
    m = jnp.mean(x, axis=axis, keepdims=True)
    v = jnp.var(x, axis=axis, keepdims=True)
    return (x - m) / jnp.sqrt(v + eps)
def _scatter_add(tgt, idx, src, axis=0):
    return tgt.at[idx].add(src)
def _segment_sum(src, seg, n):
    return jax.ops.segment_sum(src, seg, n)
class _Rng:
    def __init__(self, key):
        self._k = key
    def _next(self):
        self._k, sub = jax.random.split(self._k)
        return sub
    def normal(self, shape):
        return jax.random.normal(self._next(), shape, dtype=jnp.bfloat16)
    def randint(self, lo, hi, shape):
        return jax.random.randint(self._next(), shape, lo, hi, dtype=jnp.int32)
    def uniform(self, shape, lo=0.0, hi=1.0):
        return jax.random.uniform(self._next(), shape, jnp.bfloat16, lo, hi)
    def permutation(self, n):
        return jax.random.permutation(self._next(), n)


kernel_name = 'concat_heads__mha_block_cached__mha_block_cached__near_ridge'

def setup_inputs():
    _rng = _Rng(jax.random.key(int.from_bytes(__import__("os").urandom(4), "little")))
    _w = (lambda a: (lambda t: t.astype(jnp.bfloat16) if jnp.issubdtype(t.dtype, jnp.floating) else t)(jnp.asarray(a)))
    def _A_setup():
        B, Sq, D = 8, 160, 512
        H, Sk, Dh = 32, 512, 128
        return {
            "x": _w((lambda *s: _rng.normal(s) * 0.8)(B, Sq, D)),
            "k_cache": _w((lambda *s: _rng.normal(s) * 0.8)(B, H, Sk, Dh)),
            "v_cache": _w((lambda *s: _rng.normal(s) * 0.05)(B, H, Sk, Dh)),
            "wq": _w((lambda *s: _rng.normal(s) * 0.8)(D, H * Dh) * (D ** -0.5)),
            "wo": _w((lambda *s: _rng.normal(s) * 0.05)(H * Dh, D) * ((H * Dh) ** -0.5)),
        }
    _A_in = _A_setup()

    def _B_setup():
        B, Sq, D = 8, 160, 512
        H, Sk, Dh = 32, 512, 128
        return {
            "x": _w((lambda *s: _rng.normal(s) * 0.8)(B, Sq, D)),
            "k_cache": _w((lambda *s: _rng.normal(s) * 0.8)(B, H, Sk, Dh)),
            "v_cache": _w((lambda *s: _rng.normal(s) * 0.05)(B, H, Sk, Dh)),
            "wq": _w((lambda *s: _rng.normal(s) * 0.8)(D, H * Dh) * (D ** -0.5)),
            "wo": _w((lambda *s: _rng.normal(s) * 0.05)(H * Dh, D) * ((H * Dh) ** -0.5)),
        }
    _B_in = _B_setup()

    return {
        "A_x": _A_in["x"],
        "A_k_cache": _A_in["k_cache"],
        "A_v_cache": _A_in["v_cache"],
        "A_wq": _A_in["wq"],
        "A_wo": _A_in["wo"],
        "B_x": _B_in["x"],
        "B_k_cache": _B_in["k_cache"],
        "B_v_cache": _B_in["v_cache"],
        "B_wq": _B_in["wq"],
        "B_wo": _B_in["wo"],
    }

def reference(A_x, A_k_cache, A_v_cache, A_wq, A_wo, B_x, B_k_cache, B_v_cache, B_wq, B_wo):
    def _A_ref(x, k_cache, v_cache, wq, wo):
        B, Sq, D = x.shape
        H, Dh = 32, 128
        q = (lambda x, *d: x.transpose(*d))((x @ wq).reshape(B, Sq, H, Dh), 0, 2, 1, 3)
        scores = jnp.einsum("bhqd,bhkd->bhqk", q, k_cache) * (Dh ** -0.5)
        p = _softmax(scores, axis=-1)
        o = jnp.einsum("bhqk,bhkd->bhqd", p, v_cache)
        return (lambda x, *d: x.transpose(*d))(o, 0, 2, 1, 3).reshape(B, Sq, H * Dh) @ wo

    def _B_ref(x, k_cache, v_cache, wq, wo):
        B, Sq, D = x.shape
        H, Dh = 32, 128
        q = (lambda x, *d: x.transpose(*d))((x @ wq).reshape(B, Sq, H, Dh), 0, 2, 1, 3)
        scores = jnp.einsum("bhqd,bhkd->bhqk", q, k_cache) * (Dh ** -0.5)
        p = _softmax(scores, axis=-1)
        o = jnp.einsum("bhqk,bhkd->bhqd", p, v_cache)
        return (lambda x, *d: x.transpose(*d))(o, 0, 2, 1, 3).reshape(B, Sq, H * Dh) @ wo

    a = _A_ref(A_x, A_k_cache, A_v_cache, A_wq, A_wo)
    b = _B_ref(B_x, B_k_cache, B_v_cache, B_wq, B_wo)
    return jnp.concatenate([a, b], axis=-1)
```

```python
import functools
import jax
import jax.numpy as jnp
from jax import lax
import jax.experimental.pallas as pl
import jax.experimental.pallas.tpu as pltpu

B, SQ, D, H, SK, DH = 8, 160, 512, 32, 512, 128
LOG2E = 1.4426950408889634
f32, bf16 = jnp.float32, jnp.bfloat16

def build(U=4, UB=4, NS=16, L=15, start_at=2, flags="XLA_TPU_RESCHEDULE_DMA_DONES", nrun=64, kv_per_iter=2):
    hg = 4
    G = H // hg
    W = hg * DH
    NT = D // 128
    c = (DH ** -0.5) * LOG2E
    NSTEP = G * B
    RO = W // B
    assert NS > L and NS & (NS - 1) == 0 and NSTEP % U == 0

    def body(xa_h, ka_h, va_h, wqa_h, woa_h, xb_h, kb_h, vb_h, wqb_h, wob_h, o_h,
             x_v, k_v, v_v, wq_v, wo_v, acc, out_v, q_v, o_c,
             s_sem, p_sem, wq_sem, o_sem):
        XH, KH, VH, WQH, WOH = (xa_h, xb_h), (ka_h, kb_h), (va_h, vb_h), (wqa_h, wqb_h), (woa_h, wob_h)

        def out_copy(b):
            return pltpu.make_async_copy(out_v.at[b], o_h.at[b], o_sem.at[b])

        def payload(i, op):
            slot = i & (NS - 1)
            sem = p_sem.at[slot]
            ic = jnp.minimum(i, NSTEP - 1)
            g = lax.shift_right_logical(ic, 3); b = ic & 7
            cs = []
            for br in range(2):
                cs.append(pltpu.make_async_copy(KH[br].at[b, pl.ds(g * hg, hg)], k_v.at[br, slot], sem))
                cs.append(pltpu.make_async_copy(VH[br].at[b, pl.ds(g * hg, hg)], v_v.at[br, slot], sem))
            gw = lax.shift_right_logical(i, 3) + 1
            gs = jnp.minimum(gw, G - 1)
            gd = jnp.minimum(gw, G)
            j = i & 7
            for br in range(2):
                cs.append(pltpu.make_async_copy(WOH[br].at[pl.ds(gs * W + j * RO, RO), :], wo_v.at[br, gd, pl.ds(j * RO, RO)], sem))
            for cp in cs:
                getattr(cp, op)()

        def x_copy(br): return pltpu.make_async_copy(XH[br], x_v.at[br], s_sem.at[br])
        def wq_copy(br, g): return pltpu.make_async_copy(WQH[br].at[:, pl.ds(g * W, W)], wq_v.at[br, g], wq_sem.at[br, g])
        def wo0_copy(br): return pltpu.make_async_copy(WOH[br].at[pl.ds(0, W), :], wo_v.at[br, 0], s_sem.at[2 + br])

        def Qp(br, g, b, h):
            q = jnp.dot(x_v[br, b], wq_v[br, g, :, h * DH:(h + 1) * DH], preferred_element_type=f32)
            q_v[br, g, b, h] = (q * c).astype(bf16)

        def S(br, g, b, slot, h):
            s = lax.dot_general(q_v[br, g, b, h], k_v[br, slot, h], (((1,), (1,)), ((), ())), preferred_element_type=f32)
            m = jnp.max(s, axis=-1, keepdims=True)
            p = jnp.exp2(s - m)
            l = jnp.sum(p, axis=-1, keepdims=True)
            r = pl.reciprocal(l, approx=True)
            r = r * (2.0 - l * r)
            return p.astype(bf16), r

        def PV(br, slot, h, p, r):
            o = jnp.dot(p, v_v[br, slot, h], preferred_element_type=f32)
            return (o * r).astype(bf16)

        def Op(br, g, b, n, o):
            res = jnp.dot(o, wo_v[br, g, :, n * 128:(n + 1) * 128], preferred_element_type=f32)
            cols = pl.ds(br * D + n * 128, 128)
            t = acc[b, :, cols] + res
            acc[b, :, cols] = t
            out_v[b, :, cols] = t.astype(bf16)

        x_copy(0).start(); wq_copy(0, 0).start()
        acc[...] = jnp.zeros(acc.shape, f32)
        o_c[...] = jnp.zeros(o_c.shape, bf16)
        wo_v[1, G + 1] = jnp.zeros((W, D), bf16)
        x_copy(0).wait(); wq_copy(0, 0).wait()
        x_copy(1).start(); wq_copy(1, 0).start()
        for b in range(B):
            for h in range(hg):
                Qp(0, 0, b, h)
        x_copy(1).wait(); wq_copy(1, 0).wait()
        for gg in (1, 2):
            wq_copy(0, gg).start(); wq_copy(1, gg).start()
        for b in range(B):
            for h in range(hg):
                Qp(1, 0, b, h)

        def p1(g, carry):
            for br in range(2):
                wq_copy(br, g).wait()
            @pl.when(g + 2 < G)
            def _():
                for br in range(2):
                    wq_copy(br, g + 2).start()
            @pl.when(g == 1)
            def _():
                wo0_copy(0).start(); wo0_copy(1).start()
            for k in range(2):
                payload((g - 1) * 2 + k, "start")
            for br in range(2):
                for b in range(B):
                    for h in range(hg):
                        Qp(br, g, b, h)
            return carry
        lax.fori_loop(1, G, p1, 0)
        for i in range(2 * (G - 1), L):
            payload(jnp.int32(i), "start")
        wo0_copy(0).wait(); wo0_copy(1).wait()
        payload(jnp.int32(0), "wait")

        def step(i, do_start, last):
            g = lax.shift_right_logical(i, 3)
            b = i & 7
            slot = i & (NS - 1)
            ip = jnp.maximum(i - 1, 0); gp = jnp.where(i == 0, G + 1, lax.shift_right_logical(ip, 3)); bp = ip & 7
            pos = [0]
            def maybe_start():
                if pos[0] == start_at and do_start:
                    payload(i + L, "start")
                pos[0] += 1

            oB = jnp.concatenate([o_c[h] for h in range(hg)], axis=-1)
            pr = {}
            oA = [None] * hg
            for h in range(hg):
                maybe_start()
                pr[0, h] = S(0, g, b, slot, h)
                if h >= 1:
                    oA[h - 1] = PV(0, slot, h - 1, *pr[0, h - 1])
                Op(1, gp, bp, h, oB)
            for h in range(hg):
                maybe_start()
                pr[1, h] = S(1, g, b, slot, h)
                if h == 0:
                    oA[hg - 1] = PV(0, slot, hg - 1, *pr[0, hg - 1])
                    oAc = jnp.concatenate(oA, axis=-1)
                else:
                    o_c[h - 1] = PV(1, slot, h - 1, *pr[1, h - 1])
                    Op(0, g, b, h - 1, oAc)
            Op(0, g, b, hg - 1, oAc)
            o_c[hg - 1] = PV(1, slot, hg - 1, *pr[1, hg - 1])
            if last:
                @pl.when(i < NSTEP - 1)
                def _():
                    payload(i + 1, "wait")
            else:
                payload(i + 1, "wait")

        def loop(it, carry, do_start, U=U):
            i0 = it * U
            for u in range(U):
                step(i0 + u, do_start, (not do_start) and u == U - 1)
            @pl.when(i0 + U > (G - 1) * B)
            def _():
                for u in range(U):
                    ip = i0 + u - 1
                    @pl.when(ip >= (G - 1) * B)
                    def _():
                        out_copy(ip & 7).start()
            return carry

        NA = NSTEP - L - 1
        assert NA % U == 0 and NA % UB == 0
        lax.fori_loop(0, NA // U, functools.partial(loop, do_start=True), 0)
        payload(jnp.int32(NSTEP - 1), "start")
        lax.fori_loop(NA // UB, NSTEP // UB, functools.partial(loop, do_start=False, U=UB), 0)

        oB = jnp.concatenate([o_c[h] for h in range(hg)], axis=-1)
        for n in range(NT):
            Op(1, G - 1, B - 1, n, oB)
        out_copy(B - 1).start()
        for b in range(B):
            if nrun == NSTEP or b == B - 1:
                out_copy(b).wait()

    def fn(A_x, A_k, A_v, A_wq, A_wo, B_x, B_k, B_v, B_wq, B_wo):
        any_spec = pl.BlockSpec(memory_space=pl.ANY)
        return pl.pallas_call(
            body,
            grid=(),
            in_specs=[any_spec] * 10,
            out_specs=any_spec,
            out_shape=jax.ShapeDtypeStruct((B, SQ, 2 * D), bf16),
            scratch_shapes=[
                pltpu.VMEM((2, B, SQ, D), bf16),
                pltpu.VMEM((2, NS, hg, SK, DH), bf16),
                pltpu.VMEM((2, NS, hg, SK, DH), bf16),
                pltpu.VMEM((2, G, D, W), bf16),
                pltpu.VMEM((2, G + 2, W, D), bf16),
                pltpu.VMEM((B, SQ, 2 * D), f32),
                pltpu.VMEM((B, SQ, 2 * D), bf16),
                pltpu.VMEM((2, G, B, hg, SQ, DH), bf16),
                pltpu.VMEM((hg, SQ, DH), bf16),
                pltpu.SemaphoreType.DMA((4,)),
                pltpu.SemaphoreType.DMA((NS,)),
                pltpu.SemaphoreType.DMA((2, G)),
                pltpu.SemaphoreType.DMA((B,)),
            ],
            compiler_params=pltpu.CompilerParams(
                vmem_limit_bytes=120 * 1024 * 1024,
                flags=({k: True for k in flags.split('+')} if flags else None),
            ),
        )(A_x, A_k, A_v, A_wq, A_wo, B_x, B_k, B_v, B_wq, B_wo)
    return fn


@jax.jit
def pallas_concat_heads__mha_block_cached__mha_block_cached__near_ridge_kernel(
    A_x, A_k_cache, A_v_cache, A_wq, A_wo, B_x, B_k_cache, B_v_cache, B_wq, B_wo
):
    return build()(A_x, A_k_cache, A_v_cache, A_wq, A_wo, B_x, B_k_cache, B_v_cache, B_wq, B_wo)
```

```python
import jax
import jax.numpy as jnp
from jax import lax
import jax.experimental.pallas as pl
import jax.experimental.pallas.tpu as pltpu

B, SQ, D, H, SK, DH = 8, 160, 512, 32, 512, 128
HG = 4
G = H // HG
W = HG * DH
NT = D // 128
NSTEP = G * B
NS = 16
L = NS - 1
U = 8
NB1 = 3
RO = W // B
QSCALE = (DH ** -0.5) * 1.4426950408889634
f32, bf16 = jnp.float32, jnp.bfloat16


def _kernel(xa_h, ka_h, va_h, wqa_h, woa_h, xb_h, kb_h, vb_h, wqb_h, wob_h, o_h,
            x_v, k_v, v_v, wq_v, wo_v, acc, out_v, q_v, o_c,
            s_sem, p_sem, wq_sem, o_sem):
    XH, KH, VH, WQH, WOH = (xa_h, xb_h), (ka_h, kb_h), (va_h, vb_h), (wqa_h, wqb_h), (woa_h, wob_h)

    def step_copies(i):
        slot = i & (NS - 1)
        if isinstance(i, int):
            g, b = i // B, i % B
            g_src, g_dst = min(g + 1, G - 1), g + 1
        else:
            i = jnp.minimum(i, NSTEP - 1)
            g, b = lax.shift_right_logical(i, 3), i & (B - 1)
            g_src, g_dst = jnp.minimum(g + 1, G - 1), g + 1
        sem = p_sem.at[slot]
        cs = []
        for br in range(2):
            cs.append(pltpu.make_async_copy(KH[br].at[b, pl.ds(g * HG, HG)], k_v.at[br, slot], sem))
            cs.append(pltpu.make_async_copy(VH[br].at[b, pl.ds(g * HG, HG)], v_v.at[br, slot], sem))
        for br in range(2):
            cs.append(pltpu.make_async_copy(WOH[br].at[pl.ds(g_src * W + b * RO, RO), :],
                                            wo_v.at[br, g_dst, pl.ds(b * RO, RO)], sem))
        return cs

    def start_step(i, pred=None):
        for cp in step_copies(i):
            if pred is None:
                cp.start()
            else:
                pl.when(pred)(cp.start)

    def wait_step(i, pred=None):
        for cp in step_copies(i):
            if pred is None:
                cp.wait()
            else:
                pl.when(pred)(cp.wait)

    def xb_copy():
        return pltpu.make_async_copy(XH[1], x_v.at[1], s_sem.at[0])

    def xa_copy(lo, hi, k):
        return pltpu.make_async_copy(XH[0].at[lo:hi], x_v.at[0, lo:hi], s_sem.at[1 + k])

    def wo0_copy(br):
        return pltpu.make_async_copy(WOH[br].at[pl.ds(0, W), :], wo_v.at[br, 0], s_sem.at[3 + br])

    def wq_copy(br, g):
        return pltpu.make_async_copy(WQH[br].at[:, pl.ds(g * W, W)], wq_v.at[br, g], wq_sem.at[br, g])

    def out_copy(b):
        return pltpu.make_async_copy(out_v.at[b], o_h.at[b], o_sem.at[b])

    def last_out_copy(lo, n):
        return pltpu.make_async_copy(out_v.at[B - 1, :, pl.ds(lo, n)], o_h.at[B - 1, :, pl.ds(lo, n)],
                                     o_sem.at[B - 1])

    def q_proj(br, g, b, h):
        q = jnp.dot(x_v[br, b], wq_v[br, g, :, h * DH:(h + 1) * DH], preferred_element_type=f32)
        q_v[br, g, b, h] = (q * QSCALE).astype(bf16)

    def scores_softmax(br, g, b, slot, h):
        s = lax.dot_general(q_v[br, g, b, h], k_v[br, slot, h], (((1,), (1,)), ((), ())),
                            preferred_element_type=f32)
        m = jnp.max(s, axis=-1, keepdims=True)
        p = jnp.exp2(s - m)
        l = jnp.sum(p, axis=-1, keepdims=True)
        r = pl.reciprocal(l, approx=True)
        r = r * (2.0 - l * r)
        return p.astype(bf16), r

    def pv(br, slot, h, p, r):
        o = jnp.dot(p, v_v[br, slot, h], preferred_element_type=f32)
        return (o * r).astype(bf16)

    def o_proj(br, g, b, n, o):
        res = jnp.dot(o, wo_v[br, g, :, n * 128:(n + 1) * 128], preferred_element_type=f32)
        cols = pl.ds(br * D + n * 128, 128)
        t = acc[b, :, cols] + res
        acc[b, :, cols] = t
        out_v[b, :, cols] = t.astype(bf16)

    def seg_fetch():
        wq_copy(0, 0).start()
        xa_copy(0, NB1, 0).start()
        acc[...] = jnp.zeros(acc.shape, f32)
        xa_copy(NB1, B, 1).start()
        o_c[...] = jnp.zeros(o_c.shape, bf16)
        wo_v[1, G + 1] = jnp.zeros((W, D), bf16)

    def seg_qa_first():
        wq_copy(0, 0).wait()
        xa_copy(0, NB1, 0).wait()
        xb_copy().start()
        wq_copy(1, 0).start()
        for b in range(NB1):
            for h in range(HG):
                q_proj(0, 0, b, h)

    def seg_qa_rest():
        xa_copy(NB1, B, 1).wait()
        for b in range(NB1, B):
            for h in range(HG):
                q_proj(0, 0, b, h)

    def seg_qb():
        xb_copy().wait()
        wq_copy(1, 0).wait()
        wq_copy(0, 1).start()
        wq_copy(1, 1).start()
        for b in range(B):
            for h in range(HG):
                q_proj(1, 0, b, h)
        wq_copy(0, 2).start()
        wq_copy(1, 2).start()

    segments = (seg_fetch, seg_qa_first, seg_qa_rest, seg_qb)

    def run_segment(t, carry):
        for k, seg in enumerate(segments):
            pl.when(t == k)(seg)
        return carry

    lax.fori_loop(0, len(segments), run_segment, 0)

    def q_group(g, carry):
        for br in range(2):
            wq_copy(br, g).wait()
        for br in range(2):
            pl.when(g + 2 < G)(lambda br=br: wq_copy(br, g + 2).start())
            pl.when(g == 1)(lambda br=br: wo0_copy(br).start())
        for k in range(2):
            start_step((g - 1) * 2 + k)
        for br in range(2):
            for b in range(B):
                for h in range(HG):
                    q_proj(br, g, b, h)
        return carry

    lax.fori_loop(1, G, q_group, 0)
    for i in range(2 * (G - 1), L):
        start_step(i)
    wo0_copy(0).wait()
    wo0_copy(1).wait()
    wait_step(0)

    def step(i):
        g, b, slot = lax.shift_right_logical(i, 3), i & (B - 1), i & (NS - 1)
        ip = jnp.maximum(i - 1, 0)
        gp, bp = jnp.where(i == 0, G + 1, lax.shift_right_logical(ip, 3)), ip & (B - 1)

        o_prev = jnp.concatenate([o_c[h] for h in range(HG)], axis=-1)
        pr = {}
        o_a = [None] * HG
        for h in range(HG):
            if h == 2:
                start_step(i + L, i + L < NSTEP)
            pr[0, h] = scores_softmax(0, g, b, slot, h)
            if h >= 1:
                o_a[h - 1] = pv(0, slot, h - 1, *pr[0, h - 1])
            o_proj(1, gp, bp, h, o_prev)
        pl.when(i > NSTEP - B)(lambda: out_copy(bp).start())
        for h in range(HG):
            pr[1, h] = scores_softmax(1, g, b, slot, h)
            if h == 0:
                o_a[HG - 1] = pv(0, slot, HG - 1, *pr[0, HG - 1])
                o_a_all = jnp.concatenate(o_a, axis=-1)
            else:
                o_c[h - 1] = pv(1, slot, h - 1, *pr[1, h - 1])
                o_proj(0, g, b, h - 1, o_a_all)
        o_proj(0, g, b, HG - 1, o_a_all)
        o_c[HG - 1] = pv(1, slot, HG - 1, *pr[1, HG - 1])
        wait_step(i + 1, i + 1 < NSTEP)

    def steps(it, carry):
        for u in range(U):
            step(it * U + u)
        return carry

    lax.fori_loop(0, NSTEP // U, steps, 0)

    last_out_copy(0, D).start()
    o_prev = jnp.concatenate([o_c[h] for h in range(HG)], axis=-1)
    for n in range(NT):
        o_proj(1, G - 1, B - 1, n, o_prev)
        last_out_copy(D + n * 128, 128).start()
    for b in range(B - 1):
        out_copy(b).wait()
    last_out_copy(0, D).wait()
    for n in range(NT):
        last_out_copy(D + n * 128, 128).wait()


@jax.jit
def pallas_concat_heads__mha_block_cached__mha_block_cached__near_ridge_kernel(
    A_x: jax.Array,
    A_k_cache: jax.Array,
    A_v_cache: jax.Array,
    A_wq: jax.Array,
    A_wo: jax.Array,
    B_x: jax.Array,
    B_k_cache: jax.Array,
    B_v_cache: jax.Array,
    B_wq: jax.Array,
    B_wo: jax.Array,
):
    hbm = pl.BlockSpec(memory_space=pl.ANY)
    return pl.pallas_call(
        _kernel,
        grid=(),
        in_specs=[hbm] * 10,
        out_specs=hbm,
        out_shape=jax.ShapeDtypeStruct((B, SQ, 2 * D), bf16),
        scratch_shapes=[
            pltpu.VMEM((2, B, SQ, D), bf16),
            pltpu.VMEM((2, NS, HG, SK, DH), bf16),
            pltpu.VMEM((2, NS, HG, SK, DH), bf16),
            pltpu.VMEM((2, G, D, W), bf16),
            pltpu.VMEM((2, G + 2, W, D), bf16),
            pltpu.VMEM((B, SQ, 2 * D), f32),
            pltpu.VMEM((B, SQ, 2 * D), bf16),
            pltpu.VMEM((2, G, B, HG, SQ, DH), bf16),
            pltpu.VMEM((HG, SQ, DH), bf16),
            pltpu.SemaphoreType.DMA((5,)),
            pltpu.SemaphoreType.DMA((NS,)),
            pltpu.SemaphoreType.DMA((2, G)),
            pltpu.SemaphoreType.DMA((B,)),
        ],
        compiler_params=pltpu.CompilerParams(
            vmem_limit_bytes=110 * 1024 * 1024,
            flags={"XLA_TPU_RESCHEDULE_DMA_DONES": True},
        ),
    )(A_x, A_k_cache, A_v_cache, A_wq, A_wo, B_x, B_k_cache, B_v_cache, B_wq, B_wo)
```

```python
import jax
import jax.numpy as jnp
from jax import lax
import jax.experimental.pallas as pl
import jax.experimental.pallas.tpu as pltpu

B, SQ, D, H, SK, DH = 8, 160, 512, 32, 512, 128
HG = 4
G = H // HG
W = HG * DH
NT = D // 128
NSTEP = G * B
NS = 16
L = NS - 1
U = 8
NB1 = 3
RO = W // B
QSCALE = (DH ** -0.5) * 1.4426950408889634
f32, bf16 = jnp.float32, jnp.bfloat16


def _kernel(xa_h, ka_h, va_h, wqa_h, woa_h, xb_h, kb_h, vb_h, wqb_h, wob_h, o_h,
            x_v, k_v, v_v, wq_v, wo_v, acc, out_v, q_v, o_c,
            s_sem, p_sem, wq_sem, o_sem):
    XH, KH, VH, WQH, WOH = (xa_h, xb_h), (ka_h, kb_h), (va_h, vb_h), (wqa_h, wqb_h), (woa_h, wob_h)

    def step_copies(i):
        slot = i & (NS - 1)
        if isinstance(i, int):
            g, b = i // B, i % B
            g_src, g_dst = min(g + 1, G - 1), g + 1
        else:
            i = jnp.minimum(i, NSTEP - 1)
            g, b = lax.shift_right_logical(i, 3), i & (B - 1)
            g_src, g_dst = jnp.minimum(g + 1, G - 1), g + 1
        sem = p_sem.at[slot]
        cs = []
        for br in range(2):
            cs.append(pltpu.make_async_copy(KH[br].at[b, pl.ds(g * HG, HG)], k_v.at[br, slot], sem))
            cs.append(pltpu.make_async_copy(VH[br].at[b, pl.ds(g * HG, HG)], v_v.at[br, slot], sem))
        for br in range(2):
            cs.append(pltpu.make_async_copy(WOH[br].at[pl.ds(g_src * W + b * RO, RO), :],
                                            wo_v.at[br, g_dst, pl.ds(b * RO, RO)], sem))
        return cs

    def start_step(i, pred=None):
        for cp in step_copies(i):
            if pred is None:
                cp.start()
            else:
                pl.when(pred)(cp.start)

    def wait_step(i, pred=None):
        for cp in step_copies(i):
            if pred is None:
                cp.wait()
            else:
                pl.when(pred)(cp.wait)

    def xb_copy():
        return pltpu.make_async_copy(XH[1], x_v.at[1], s_sem.at[0])

    def xa_copy(lo, hi, k):
        return pltpu.make_async_copy(XH[0].at[lo:hi], x_v.at[0, lo:hi], s_sem.at[1 + k])

    def wo0_copy(br):
        return pltpu.make_async_copy(WOH[br].at[pl.ds(0, W), :], wo_v.at[br, 0], s_sem.at[3 + br])

    def wq_copy(br, g):
        return pltpu.make_async_copy(WQH[br].at[:, pl.ds(g * W, W)], wq_v.at[br, g], wq_sem.at[br, g])

    def out_copy(b):
        return pltpu.make_async_copy(out_v.at[b], o_h.at[b], o_sem.at[b])

    def last_out_copy(lo, n):
        return pltpu.make_async_copy(out_v.at[B - 1, :, pl.ds(lo, n)], o_h.at[B - 1, :, pl.ds(lo, n)],
                                     o_sem.at[B - 1])

    def q_proj(br, g, b, h):
        q = jnp.dot(x_v[br, b], wq_v[br, g, :, h * DH:(h + 1) * DH], preferred_element_type=f32)
        q_v[br, g, b, h] = (q * QSCALE).astype(bf16)

    def scores_softmax(br, g, b, slot, h):
        s = lax.dot_general(q_v[br, g, b, h], k_v[br, slot, h], (((1,), (1,)), ((), ())),
                            preferred_element_type=f32)
        m = jnp.max(s, axis=-1, keepdims=True)
        p = jnp.exp2(s - m)
        l = jnp.sum(p, axis=-1, keepdims=True)
        r = pl.reciprocal(l, approx=True)
        r = r * (2.0 - l * r)
        return p.astype(bf16), r

    def pv(br, slot, h, p, r):
        o = jnp.dot(p, v_v[br, slot, h], preferred_element_type=f32)
        return (o * r).astype(bf16)

    def o_proj(br, g, b, n, o):
        res = jnp.dot(o, wo_v[br, g, :, n * 128:(n + 1) * 128], preferred_element_type=f32)
        cols = pl.ds(br * D + n * 128, 128)
        t = acc[b, :, cols] + res
        acc[b, :, cols] = t
        out_v[b, :, cols] = t.astype(bf16)

    def seg_fetch():
        wq_copy(0, 0).start()
        xa_copy(0, NB1, 0).start()
        acc[...] = jnp.zeros(acc.shape, f32)
        xa_copy(NB1, B, 1).start()
        o_c[...] = jnp.zeros(o_c.shape, bf16)
        wo_v[1, G + 1] = jnp.zeros((W, D), bf16)

    def seg_qa_first():
        wq_copy(0, 0).wait()
        xa_copy(0, NB1, 0).wait()
        xb_copy().start()
        wq_copy(1, 0).start()
        for b in range(NB1):
            for h in range(HG):
                q_proj(0, 0, b, h)

    def seg_qa_rest():
        xa_copy(NB1, B, 1).wait()
        for b in range(NB1, B):
            for h in range(HG):
                q_proj(0, 0, b, h)

    def seg_qb():
        xb_copy().wait()
        wq_copy(1, 0).wait()
        wq_copy(0, 1).start()
        wq_copy(1, 1).start()
        for b in range(B):
            for h in range(HG):
                q_proj(1, 0, b, h)
        wq_copy(0, 2).start()
        wq_copy(1, 2).start()

    segments = (seg_fetch, seg_qa_first, seg_qa_rest, seg_qb)

    def run_segment(t, carry):
        for k, seg in enumerate(segments):
            pl.when(t == k)(seg)
        return carry

    lax.fori_loop(0, len(segments), run_segment, 0)

    def q_group(g, carry):
        for br in range(2):
            wq_copy(br, g).wait()
        for br in range(2):
            pl.when(g + 2 < G)(lambda br=br: wq_copy(br, g + 2).start())
            pl.when(g == 1)(lambda br=br: wo0_copy(br).start())
        for k in range(2):
            start_step((g - 1) * 2 + k)
        for br in range(2):
            for b in range(B):
                for h in range(HG):
                    q_proj(br, g, b, h)
        return carry

    lax.fori_loop(1, G, q_group, 0)
    for i in range(2 * (G - 1), L):
        start_step(i)
    wo0_copy(0).wait()
    wo0_copy(1).wait()
    wait_step(0)

    def step(i):
        g, b, slot = lax.shift_right_logical(i, 3), i & (B - 1), i & (NS - 1)
        ip = jnp.maximum(i - 1, 0)
        gp, bp = jnp.where(i == 0, G + 1, lax.shift_right_logical(ip, 3)), ip & (B - 1)

        o_prev = jnp.concatenate([o_c[h] for h in range(HG)], axis=-1)
        probs, o_a = {}, [None] * HG

        def sc(br, h):
            probs[br, h] = scores_softmax(br, g, b, slot, h)

        def pv_a(h):
            o_a[h] = pv(0, slot, h, *probs[0, h])

        def pv_b(h):
            o_c[h] = pv(1, slot, h, *probs[1, h])

        def o_b(n):
            o_proj(1, gp, bp, n, o_prev)

        o_b(0); sc(0, 0); o_b(1)
        start_step(i + L, i + L < NSTEP)
        sc(0, 1); o_b(2); sc(0, 2); pv_a(0); sc(0, 3); pv_a(1); o_b(3)
        pl.when(i > NSTEP - B)(lambda: out_copy(bp).start())
        sc(1, 0); pv_a(2); sc(1, 1); pv_a(3)
        o_a_all = jnp.concatenate(o_a, axis=-1)
        o_proj(0, g, b, 0, o_a_all); sc(1, 2); pv_b(0)
        o_proj(0, g, b, 1, o_a_all); sc(1, 3); pv_b(1)
        o_proj(0, g, b, 2, o_a_all); pv_b(2); pv_b(3)
        o_proj(0, g, b, 3, o_a_all)
        wait_step(i + 1, i + 1 < NSTEP)

    def steps(it, carry):
        for u in range(U):
            step(it * U + u)
        return carry

    lax.fori_loop(0, NSTEP // U, steps, 0)

    last_out_copy(0, D).start()
    o_prev = jnp.concatenate([o_c[h] for h in range(HG)], axis=-1)
    for n in range(NT):
        o_proj(1, G - 1, B - 1, n, o_prev)
        last_out_copy(D + n * 128, 128).start()
    for b in range(B - 1):
        out_copy(b).wait()
    last_out_copy(0, D).wait()
    for n in range(NT):
        last_out_copy(D + n * 128, 128).wait()


@jax.jit
def pallas_concat_heads__mha_block_cached__mha_block_cached__near_ridge_kernel(
    A_x: jax.Array,
    A_k_cache: jax.Array,
    A_v_cache: jax.Array,
    A_wq: jax.Array,
    A_wo: jax.Array,
    B_x: jax.Array,
    B_k_cache: jax.Array,
    B_v_cache: jax.Array,
    B_wq: jax.Array,
    B_wo: jax.Array,
):
    hbm = pl.BlockSpec(memory_space=pl.ANY)
    return pl.pallas_call(
        _kernel,
        grid=(),
        in_specs=[hbm] * 10,
        out_specs=hbm,
        out_shape=jax.ShapeDtypeStruct((B, SQ, 2 * D), bf16),
        scratch_shapes=[
            pltpu.VMEM((2, B, SQ, D), bf16),
            pltpu.VMEM((2, NS, HG, SK, DH), bf16),
            pltpu.VMEM((2, NS, HG, SK, DH), bf16),
            pltpu.VMEM((2, G, D, W), bf16),
            pltpu.VMEM((2, G + 2, W, D), bf16),
            pltpu.VMEM((B, SQ, 2 * D), f32),
            pltpu.VMEM((B, SQ, 2 * D), bf16),
            pltpu.VMEM((2, G, B, HG, SQ, DH), bf16),
            pltpu.VMEM((HG, SQ, DH), bf16),
            pltpu.SemaphoreType.DMA((5,)),
            pltpu.SemaphoreType.DMA((NS,)),
            pltpu.SemaphoreType.DMA((2, G)),
            pltpu.SemaphoreType.DMA((B,)),
        ],
        compiler_params=pltpu.CompilerParams(
            vmem_limit_bytes=110 * 1024 * 1024,
            flags={"XLA_TPU_RESCHEDULE_DMA_DONES": True},
        ),
    )(A_x, A_k_cache, A_v_cache, A_wq, A_wo, B_x, B_k_cache, B_v_cache, B_wq, B_wo)
```

```python
import jax
import jax.numpy as jnp
from jax import lax
import jax.experimental.pallas as pl
import jax.experimental.pallas.tpu as pltpu

B, SQ, D, H, SK, DH = 8, 160, 512, 32, 512, 128
HG = 4
G = H // HG
W = HG * DH
NT = D // 128
NSTEP = G * B
NS = 16
L = NS - 1
U = 8
NB1 = 3
RO = W // B
QSCALE = (DH ** -0.5) * 1.4426950408889634
f32, bf16 = jnp.float32, jnp.bfloat16


def _kernel(xa_h, ka_h, va_h, wqa_h, woa_h, xb_h, kb_h, vb_h, wqb_h, wob_h, o_h,
            x_v, k_v, v_v, w_v, acc, out_v, q_v, o_c,
            s_sem, p_sem, wq_sem, o_sem):
    XH, KH, VH, WQH, WOH = (xa_h, xb_h), (ka_h, kb_h), (va_h, vb_h), (wqa_h, wqb_h), (woa_h, wob_h)

    def step_copies(i):
        slot = i & (NS - 1)
        if isinstance(i, int):
            g, b = i // B, i % B
            g_src, g_dst = min(g + 1, G - 1), g + 1
        else:
            i = jnp.minimum(i, NSTEP - 1)
            g, b = lax.shift_right_logical(i, 3), i & (B - 1)
            g_src, g_dst = jnp.minimum(g + 1, G - 1), g + 1
        sem = p_sem.at[slot]
        cs = []
        for br in range(2):
            cs.append(pltpu.make_async_copy(KH[br].at[b, pl.ds(g * HG, HG)], k_v.at[br, slot], sem))
            cs.append(pltpu.make_async_copy(VH[br].at[b, pl.ds(g * HG, HG)], v_v.at[br, slot], sem))
        for br in range(2):
            cs.append(pltpu.make_async_copy(WOH[br].at[pl.ds(g_src * W + b * RO, RO), :],
                                            w_v.at[br, G + g_dst, pl.ds(b * RO, RO)], sem))
        return cs

    def start_step(i, pred=None):
        for cp in step_copies(i):
            if pred is None:
                cp.start()
            else:
                pl.when(pred)(cp.start)

    def wait_step(i, pred=None):
        for cp in step_copies(i):
            if pred is None:
                cp.wait()
            else:
                pl.when(pred)(cp.wait)

    def xb_copy():
        return pltpu.make_async_copy(XH[1], x_v.at[1], s_sem.at[2])

    def xa_copy(lo, hi, k):
        return pltpu.make_async_copy(XH[0].at[lo:hi], x_v.at[0, lo:hi], s_sem.at[k])

    def wo0_copy(br):
        return pltpu.make_async_copy(WOH[br].at[pl.ds(0, W), :], w_v.at[br, G], s_sem.at[0])

    def wq_copy(br, g, sem=None):
        sem = wq_sem.at[g & 1] if sem is None else sem
        return pltpu.make_async_copy(WQH[br].at[:, pl.ds(g * W, W)], w_v.at[br, g], sem)

    def out_copy(b):
        return pltpu.make_async_copy(out_v.at[b], o_h.at[b], o_sem)

    def last_out_copy(lo, n):
        return pltpu.make_async_copy(out_v.at[B - 1, :, pl.ds(lo, n)], o_h.at[B - 1, :, pl.ds(lo, n)], o_sem)

    def q_proj(br, g, b, h):
        q = jnp.dot(x_v[br, b], w_v[br, g, :, h * DH:(h + 1) * DH], preferred_element_type=f32)
        q_v[br, g, b, h] = (q * QSCALE).astype(bf16)

    def scores_softmax(br, q, slot, h):
        s = lax.dot_general(q, k_v[br, slot, h], (((1,), (1,)), ((), ())),
                            preferred_element_type=f32)
        m = jnp.max(s, axis=-1, keepdims=True)
        p = jnp.exp2(s - m)
        l = jnp.sum(p, axis=-1, keepdims=True)
        r = pl.reciprocal(l, approx=True)
        r = r * (2.0 - l * r)
        return p.astype(bf16), r

    def pv(br, slot, h, p, r):
        o = jnp.dot(p, v_v[br, slot, h], preferred_element_type=f32)
        return (o * r).astype(bf16)

    def o_proj(br, w, b, n, o):
        res = jnp.dot(o, w_v[br, w, :, n * 128:(n + 1) * 128], preferred_element_type=f32)
        cols = pl.ds(br * D + n * 128, 128)
        t = acc[b, :, cols] + res
        acc[b, :, cols] = t
        out_v[b, :, cols] = t.astype(bf16)
        return t

    def seg_fetch():
        wq_copy(0, 0, s_sem.at[0]).start()
        xa_copy(0, NB1, 0).start()
        acc[...] = jnp.zeros(acc.shape, f32)
        xa_copy(NB1, B, 1).start()

    def seg_qa_first():
        wq_copy(0, 0, s_sem.at[0]).wait()
        xa_copy(0, NB1, 0).wait()
        xb_copy().start()
        wq_copy(1, 0, s_sem.at[2]).start()
        for b in range(NB1):
            for h in range(HG):
                q_proj(0, 0, b, h)

    def seg_qa_rest():
        xa_copy(NB1, B, 1).wait()
        for b in range(NB1, B):
            for h in range(HG):
                q_proj(0, 0, b, h)

    def seg_qb():
        xb_copy().wait()
        wq_copy(1, 0, s_sem.at[2]).wait()
        wq_copy(0, 1).start()
        wq_copy(1, 1).start()
        for k in range(NT):
            o_c[k] = x_v[1, 0, :, k * 128:(k + 1) * 128]
        q_v[1, 0, 0] = jnp.zeros(q_v.shape[3:], bf16)
        for b in range(1, B):
            for h in range(HG):
                q_proj(1, 0, b, h)
        wq_copy(0, 2).start()
        wq_copy(1, 2).start()

    segments = (seg_fetch, seg_qa_first, seg_qa_rest, seg_qb)

    def run_segment(t, carry):
        for k, seg in enumerate(segments):
            pl.when(t == k)(seg)
        return carry

    lax.fori_loop(0, len(segments), run_segment, 0)

    def q_group(g, carry):
        for br in range(2):
            wq_copy(br, g).wait()
        for br in range(2):
            pl.when(g + 2 < G)(lambda br=br: wq_copy(br, g + 2).start())
            pl.when(g == 1)(lambda br=br: wo0_copy(br).start())
        for k in range(2):
            start_step((g - 1) * 2 + k)
        for br in range(2):
            for b in range(B):
                for h in range(HG):
                    q_proj(br, g, b, h)
        return carry

    lax.fori_loop(1, G, q_group, 0)
    for i in range(2 * (G - 1), L):
        start_step(i)
    wo0_copy(0).wait()
    wo0_copy(1).wait()
    wait_step(0)

    def step(i):
        g, b, slot = lax.shift_right_logical(i, 3), i & (B - 1), i & (NS - 1)
        ip = jnp.maximum(i - 1, 0)
        first = i == 0
        wp = jnp.where(first, 0, G + lax.shift_right_logical(ip, 3))
        bp = jnp.where(first, B, ip & (B - 1))

        o_prev = jnp.concatenate([o_c[h] for h in range(HG)], axis=-1)
        probs, o_a, q_first = {}, [None] * HG, [None] * HG

        def sc(br, h):
            q = q_v[br, g, b, h]
            if br == 1:
                q = jnp.where(first, q_first[h], q)
            probs[br, h] = scores_softmax(br, q, slot, h)

        def pv_a(h):
            o_a[h] = pv(0, slot, h, *probs[0, h])

        def pv_b(h):
            o_c[h] = pv(1, slot, h, *probs[1, h])

        def o_b(n):
            t = o_proj(1, wp, bp, n, o_prev)
            q_first[n] = (t * QSCALE).astype(bf16)

        o_b(0); sc(0, 0); o_b(1)
        start_step(i + L, i + L < NSTEP)
        sc(0, 1); o_b(2); sc(0, 2); pv_a(0); sc(0, 3); pv_a(1); o_b(3)
        pl.when(i > NSTEP - B)(lambda: out_copy(ip & (B - 1)).start())
        sc(1, 0); pv_a(2); sc(1, 1); pv_a(3)
        o_a_all = jnp.concatenate(o_a, axis=-1)
        o_proj(0, G + g, b, 0, o_a_all); sc(1, 2); pv_b(0)
        o_proj(0, G + g, b, 1, o_a_all); sc(1, 3); pv_b(1)
        o_proj(0, G + g, b, 2, o_a_all); pv_b(2); pv_b(3)
        o_proj(0, G + g, b, 3, o_a_all)
        wait_step(i + 1, i + 1 < NSTEP)

    def steps(it, carry):
        for u in range(U):
            step(it * U + u)
        return carry

    lax.fori_loop(0, NSTEP // U, steps, 0)

    last_out_copy(0, D).start()
    o_prev = jnp.concatenate([o_c[h] for h in range(HG)], axis=-1)
    for n in range(NT):
        o_proj(1, 2 * G - 1, B - 1, n, o_prev)
        last_out_copy(D + n * 128, 128).start()
    pltpu.make_async_copy(o_h, o_h, o_sem).wait()


@jax.jit
def pallas_concat_heads__mha_block_cached__mha_block_cached__near_ridge_kernel(
    A_x: jax.Array,
    A_k_cache: jax.Array,
    A_v_cache: jax.Array,
    A_wq: jax.Array,
    A_wo: jax.Array,
    B_x: jax.Array,
    B_k_cache: jax.Array,
    B_v_cache: jax.Array,
    B_wq: jax.Array,
    B_wo: jax.Array,
):
    hbm = pl.BlockSpec(memory_space=pl.ANY)
    return pl.pallas_call(
        _kernel,
        grid=(),
        in_specs=[hbm] * 10,
        out_specs=hbm,
        out_shape=jax.ShapeDtypeStruct((B, SQ, 2 * D), bf16),
        scratch_shapes=[
            pltpu.VMEM((2, B, SQ, D), bf16),
            pltpu.VMEM((2, NS, HG, SK, DH), bf16),
            pltpu.VMEM((2, NS, HG, SK, DH), bf16),
            pltpu.VMEM((2, 2 * G + 1, D, W), bf16),
            pltpu.VMEM((B + 1, SQ, 2 * D), f32),
            pltpu.VMEM((B + 1, SQ, 2 * D), bf16),
            pltpu.VMEM((2, G, B, HG, SQ, DH), bf16),
            pltpu.VMEM((HG, SQ, DH), bf16),
            pltpu.SemaphoreType.DMA((3,)),
            pltpu.SemaphoreType.DMA((NS,)),
            pltpu.SemaphoreType.DMA((2,)),
            pltpu.SemaphoreType.DMA(()),
        ],
        compiler_params=pltpu.CompilerParams(
            vmem_limit_bytes=110 * 1024 * 1024,
            flags={"XLA_TPU_RESCHEDULE_DMA_DONES": True},
        ),
    )(A_x, A_k_cache, A_v_cache, A_wq, A_wo, B_x, B_k_cache, B_v_cache, B_wq, B_wo)
```
